```python
import os as _os
_os.environ.setdefault("JAX_PLATFORMS", "cpu")
import jax
import jax.numpy as jnp

def _softmax(x, axis=-1):
    return jax.nn.softmax(x, axis=axis)
def _gelu(x):
    return jax.nn.gelu(x, approximate=True)
def _silu(x):
    return jax.nn.silu(x)
def _sigmoid(x):
    return jax.nn.sigmoid(x)
def _layernorm(x, axis=-1, eps=1e-5):
    m = jnp.mean(x, axis=axis, keepdims=True)
    v = jnp.var(x, axis=axis, keepdims=True)
    return (x - m) / jnp.sqrt(v + eps)
def _scatter_add(tgt, idx, src, axis=0):
    return tgt.at[idx].add(src)
def _segment_sum(src, seg, n):
    return jax.ops.segment_sum(src, seg, n)
class _Rng:
    def __init__(self, key):
        self._k = key
    def _next(self):
        self._k, sub = jax.random.split(self._k)
        return sub
    def normal(self, shape):
        return jax.random.normal(self._next(), shape, dtype=jnp.bfloat16)
    def randint(self, lo, hi, shape):
        return jax.random.randint(self._next(), shape, lo, hi, dtype=jnp.int32)
    def uniform(self, shape, lo=0.0, hi=1.0):
        return jax.random.uniform(self._next(), shape, jnp.bfloat16, lo, hi)
    def permutation(self, n):
        return jax.random.permutation(self._next(), n)


kernel_name = 'sequential_preLN__linear_attn_block__dense_activation_squared_relu__prompt'

def setup_inputs():
    _rng = _Rng(jax.random.key(int.from_bytes(__import__("os").urandom(4), "little")))
    _w = (lambda a: (lambda t: t.astype(jnp.bfloat16) if jnp.issubdtype(t.dtype, jnp.floating) else t)(jnp.asarray(a)))
    def _A_setup():
        B, S, D = 1, 2048, 576
        return {
            "x": _w((lambda *s: _rng.normal(s) * 0.05)(B, S, D)),
            "wqkv": _w((lambda *s: _rng.normal(s) * 0.1)(D, 3 * D)),
            "wo": _w((lambda *s: _rng.normal(s) * 0.05)(D, D)),
        }
    _A_in = _A_setup()

    def _B_setup():
        B, S, D, F = 1, 2048, 576, 4608
        return {
            "x": _w((lambda *s: _rng.normal(s) * 0.05)(B, S, D)),
            "w1": _w((lambda *s: _rng.normal(s) * 0.05)(D, F)),
            "b1": _w((lambda *s: _rng.normal(s) * 0.05)(F)),
            "w2": _w((lambda *s: _rng.normal(s) * 0.05)(F, D)),
            "b2": _w((lambda *s: _rng.normal(s) * 0.05)(D)),
        }
    _B_in = _B_setup()

    return {
        "A_x": _A_in["x"],
        "A_wqkv": _A_in["wqkv"],
        "A_wo": _A_in["wo"],
        "B_x": _B_in["x"],
        "B_w1": _B_in["w1"],
        "B_b1": _B_in["b1"],
        "B_w2": _B_in["w2"],
        "B_b2": _B_in["b2"],
    }

def reference(A_x, A_wqkv, A_wo, B_x, B_w1, B_b1, B_w2, B_b2):
    def _A_ref(x, wqkv, wo):
        B, S, D = x.shape
        H = 32; Dh = D // H
        qkv = (lambda x, *d: x.transpose(*d))((x @ wqkv).reshape(B, S, 3, H, Dh), 2, 0, 3, 1, 4)
        q, k, v = qkv[0], qkv[1], qkv[2]
        phi = lambda t: jnp.where(t > 0, t + 1, jnp.exp(t)) + 1e-6
        pq, pk = phi(q), phi(k)
        kv = jnp.einsum("bhsd,bhse->bhde", pk, v)
        z = jnp.einsum("bhsd->bhd", pk)
        num = jnp.einsum("bhqd,bhde->bhqe", pq, kv)
        den = jnp.einsum("bhqd,bhd->bhq", pq, z)[..., None] + 1e-6
        o = num / den
        return (lambda x, *d: x.transpose(*d))(o, 0, 2, 1, 3).reshape(B, S, D) @ wo

    def _B_ref(x, w1, b1, w2, b2):
        h = jnp.einsum("bsd,df->bsf", x, w1) + b1
        zero = jnp.zeros_like(h)
        r = jnp.where(h > zero, h, zero)
        h = r * r
        out = jnp.einsum("bsf,fd->bsd", h, w2) + b2
        return out

    x = A_x
    h = x + _A_ref(_layernorm(x, axis=-1), A_wqkv, A_wo)
    h2 = h + _B_ref(_layernorm(h, axis=-1), B_w1, B_b1, B_w2, B_b2)
    return h2
```

```python
import functools

import jax
import jax.numpy as jnp
from jax import lax
import jax.experimental.pallas as pl
import jax.experimental.pallas.tpu as pltpu

_LN_EPS = 1e-5
_PHI_EPS = 1e-6
_DEN_EPS = 1e-6
_NUM_HEADS = 32
_LANE = 128


def _round_up(a, b):
    return (a + b - 1) // b * b


def _layernorm_f32(x):
    m = jnp.mean(x, axis=-1, keepdims=True)
    xc = x - m
    v = jnp.mean(xc * xc, axis=-1, keepdims=True)
    return xc * lax.rsqrt(v + _LN_EPS)


def _head_of(idx, dh):
    return jnp.floor((idx.astype(jnp.float32) + 0.5) * (1.0 / dh)).astype(jnp.int32)


def _kernel(x_ref, wqkv_ref, wo_ref, b1_ref, b2_ref, w1_hbm, w2_hbm, o_ref,
            w1_v, w2_v, sems, pq_s, kv_s, m_s, z_s,
            *, n_tiles, tm, d, dp, f, fc, heads):
    i = pl.program_id(0)
    dh = d // heads
    pad = dp - d
    k_lo = d - pad

    def w1_copy():
        return pltpu.make_async_copy(w1_hbm, w1_v, sems.at[0])

    def w2_copy():
        return pltpu.make_async_copy(w2_hbm, w2_v, sems.at[1])

    @pl.when(i == 0)
    def _():
        w1_copy().start()
        w2_copy().start()
        kv_s[...] = jnp.zeros(kv_s.shape, kv_s.dtype)

    @pl.when(i < n_tiles)
    def _():
        xn = _layernorm_f32(x_ref[...].astype(jnp.float32)).astype(jnp.bfloat16)
        qkv = jnp.dot(xn, wqkv_ref[...], preferred_element_type=jnp.float32)
        qk = qkv[:, :2 * d]
        pqk = (jnp.where(qk > 0, qk + 1.0, jnp.exp(qk)) + _PHI_EPS).astype(jnp.bfloat16)
        vv = qkv[:, 2 * d:]
        col = lax.broadcasted_iota(jnp.int32, vv.shape, 1)
        v_aug = jnp.where(col < d, vv, 1.0).astype(jnp.bfloat16)
        start = pl.multiple_of(i * tm, tm)
        pq_s[pl.ds(start, tm), :] = pqk[:, :dp]
        kv_s[...] += lax.dot_general(
            pqk[:, k_lo:], v_aug, (((0,), (0,)), ((), ())),
            preferred_element_type=jnp.float32)

    @pl.when(i == n_tiles - 1)
    def _():
        kv = kv_s[pad:, :]
        row = lax.broadcasted_iota(jnp.int32, kv.shape, 0)
        col = lax.broadcasted_iota(jnp.int32, kv.shape, 1)
        hr = _head_of(row, dh)
        hc = jnp.where(col < d, _head_of(col, dh), (col - d) & (heads - 1))
        r = jnp.where(hr == hc, kv, 0.0).astype(jnp.bfloat16)
        m = jnp.dot(r[:, :d], wo_ref[...], preferred_element_type=jnp.float32)
        m_s[:d, :] = m.astype(jnp.bfloat16)
        m_s[d:, :] = jnp.zeros((pad, d), jnp.bfloat16)
        z_s[:d, :] = r[:, k_lo:]
        z_s[d:, :] = jnp.zeros((pad, _LANE), jnp.bfloat16)

    @pl.when(i >= n_tiles)
    def _():
        @pl.when(i == n_tiles)
        def _():
            w1_copy().wait()
            w2_copy().wait()

        start = pl.multiple_of((i - n_tiles) * tm, tm)
        pq = pq_s[pl.ds(start, tm), :]
        den = jnp.dot(pq, z_s[...], preferred_element_type=jnp.float32)
        lane = lax.broadcasted_iota(jnp.int32, den.shape, 1)
        rec = 1.0 / (den + _DEN_EPS)
        rec_hi = rec.astype(jnp.bfloat16).astype(jnp.float32)
        r2 = jnp.where(lane < pad, 0.0,
                       jnp.where(lane < pad + heads, rec_hi, rec - rec_hi))
        erow = lax.broadcasted_iota(jnp.int32, (_LANE, dp), 0)
        ecol = lax.broadcasted_iota(jnp.int32, (_LANE, dp), 1)
        expand = jnp.where(
            (erow >= pad) & (ecol < d)
            & (((erow - pad) & (heads - 1)) == _head_of(ecol, dh)),
            1.0, 0.0).astype(jnp.bfloat16)
        rb = jnp.dot(r2.astype(jnp.bfloat16), expand,
                     preferred_element_type=jnp.float32)
        pqs = (pq.astype(jnp.float32) * rb).astype(jnp.bfloat16)
        attn = jnp.dot(pqs, m_s[...], preferred_element_type=jnp.float32)
        h = x_ref[...].astype(jnp.float32) + attn
        hn = _layernorm_f32(h).astype(jnp.bfloat16)
        acc = h + b2_ref[...].astype(jnp.float32)
        for c in range(f // fc):
            a = jnp.dot(hn, w1_v[:, c * fc:(c + 1) * fc],
                        preferred_element_type=jnp.float32)
            a = a + b1_ref[:, c * fc:(c + 1) * fc].astype(jnp.float32)
            a = jnp.maximum(a, 0.0)
            a = (a * a).astype(jnp.bfloat16)
            acc = acc + jnp.dot(a, w2_v[c * fc:(c + 1) * fc, :],
                                preferred_element_type=jnp.float32)
        o_ref[...] = acc.astype(o_ref.dtype)


@jax.jit
def pallas_sequential_preLN__linear_attn_block__dense_activation_squared_relu__prompt_kernel(
    A_x: jax.Array,
    A_wqkv: jax.Array,
    A_wo: jax.Array,
    B_x: jax.Array,
    B_w1: jax.Array,
    B_b1: jax.Array,
    B_w2: jax.Array,
    B_b2: jax.Array,
):
    del B_x
    b, s, d = A_x.shape
    assert b == 1
    f = B_w1.shape[1]
    dp = _round_up(d, _LANE)
    assert dp - d == 2 * _NUM_HEADS and (2 * d) % _LANE == 0
    tm = 256
    fc = 512
    assert s % tm == 0 and f % fc == 0
    n_tiles = s // tm

    x2 = A_x.reshape(s, d)
    b1 = B_b1.reshape(1, f)
    b2 = B_b2.reshape(1, d)

    kernel = functools.partial(
        _kernel, n_tiles=n_tiles, tm=tm, d=d, dp=dp, f=f, fc=fc, heads=_NUM_HEADS)

    out = pl.pallas_call(
        kernel,
        grid=(2 * n_tiles,),
        in_specs=[
            pl.BlockSpec((tm, d), lambda i: (i % n_tiles, 0)),
            pl.BlockSpec((d, 2 * d + dp), lambda i: (0, 0)),
            pl.BlockSpec((d, d), lambda i: (0, 0)),
            pl.BlockSpec((1, f), lambda i: (0, 0)),
            pl.BlockSpec((1, d), lambda i: (0, 0)),
            pl.BlockSpec(memory_space=pl.ANY),
            pl.BlockSpec(memory_space=pl.ANY),
        ],
        out_specs=pl.BlockSpec((tm, d), lambda i: (jnp.maximum(i - n_tiles, 0), 0)),
        out_shape=jax.ShapeDtypeStruct((s, d), A_x.dtype),
        scratch_shapes=[
            pltpu.VMEM((d, f), jnp.bfloat16),
            pltpu.VMEM((f, d), jnp.bfloat16),
            pltpu.SemaphoreType.DMA((2,)),
            pltpu.VMEM((s, dp), jnp.bfloat16),
            pltpu.VMEM((dp, dp), jnp.float32),
            pltpu.VMEM((dp, d), jnp.bfloat16),
            pltpu.VMEM((dp, _LANE), jnp.bfloat16),
        ],
        compiler_params=pltpu.CompilerParams(
            dimension_semantics=("arbitrary",),
            vmem_limit_bytes=100 * 1024 * 1024,
        ),
    )(x2, A_wqkv, A_wo, b1, b2, B_w1, B_w2)
    return out.reshape(b, s, d)
```

```python
import functools

import jax
import jax.numpy as jnp
from jax import lax
import jax.experimental.pallas as pl
import jax.experimental.pallas.tpu as pltpu

_LN_EPS = 1e-5
_PHI_EPS = 1e-6
_DEN_EPS = 1e-6
_NUM_HEADS = 32
_LANE = 128

_NT = (((1,), (1,)), ((), ()))
_TN = (((0,), (0,)), ((), ()))


def _round_up(a, b):
    return (a + b - 1) // b * b


def _layernorm_cols(x):
    m = jnp.mean(x, axis=0, keepdims=True)
    xc = x - m
    v = jnp.mean(xc * xc, axis=0, keepdims=True)
    return xc * lax.rsqrt(v + _LN_EPS)


def _head_of(idx, dh):
    return jnp.floor((idx.astype(jnp.float32) + 0.5) * (1.0 / dh)).astype(jnp.int32)


def _head_blocks(d, dh):
    blocks = []
    for c0 in range(0, d, _LANE):
        c1 = min(c0 + _LANE, d)
        r0 = (c0 // dh) * dh // 16 * 16
        r1 = min(_round_up(((c1 - 1) // dh + 1) * dh, 16), d)
        blocks.append((r0, r1, c0, c1))
    return blocks


def _kernel(b1_ref, b2_ref, x_hbm, wqkv_hbm, wo_hbm, w1_hbm, w2t_hbm, o_ref,
            x_v, wqkv_v, wo_v, w1_v, w2t_v, x_sems, wqkv_sems, sems,
            wqkvt_s, pq_s, kvt_s, zsum_s, mt_s, zt_s, b2_s,
            *, n_tiles, ts, d, dp, f, fc, wqc, heads):
    i = pl.program_id(0)
    dh = d // heads
    pad = dp - d
    blocks = _head_blocks(d, dh)
    wq_chunks = [(c, min(c + wqc, 3 * d)) for c in range(0, 3 * d, wqc)]

    def x_copy(t):
        return pltpu.make_async_copy(
            x_hbm.at[:, pl.ds(t * ts, ts)], x_v.at[:, pl.ds(t * ts, ts)], x_sems.at[t])

    def wqkv_copy(j):
        c0, c1 = wq_chunks[j]
        return pltpu.make_async_copy(
            wqkv_hbm.at[:, pl.ds(c0, c1 - c0)], wqkv_v.at[:, pl.ds(c0, c1 - c0)],
            wqkv_sems.at[j])

    def wo_copy():
        return pltpu.make_async_copy(wo_hbm, wo_v, sems.at[2])

    def w1_copy():
        return pltpu.make_async_copy(w1_hbm, w1_v.at[pl.ds(0, d), :], sems.at[0])

    def w2_copy():
        return pltpu.make_async_copy(w2t_hbm, w2t_v, sems.at[1])

    @pl.when(i == 0)
    def _():
        wqkv_copy(0).start()
        wqkv_copy(1).start()
        kvt_s[...] = jnp.zeros(kvt_s.shape, kvt_s.dtype)
        zsum_s[...] = jnp.zeros(zsum_s.shape, zsum_s.dtype)
        prow = lax.broadcasted_iota(jnp.int32, (pad, f), 0)
        w1_v[d:, :] = jnp.where(
            prow == 0, b1_ref[...].astype(jnp.float32).reshape(1, f), 0.0
        ).astype(jnp.bfloat16)
        b2_s[...] = jnp.broadcast_to(
            b2_ref[...].astype(jnp.float32).reshape(1, d), (_LANE, d)).T
        for j, (c0, c1) in enumerate(wq_chunks):
            wqkv_copy(j).wait()
            if j + 2 < len(wq_chunks):
                wqkv_copy(j + 2).start()
            if j + 2 == len(wq_chunks):
                x_copy(0).start()
            wqkvt_s[c0:c1, :] = (
                wqkv_v[:, c0:c1].astype(jnp.float32).T.astype(jnp.bfloat16))
        x_copy(0).wait()
        for t in range(1, n_tiles):
            x_copy(t).start()
        wo_copy().start()
        w1_copy().start()
        w2_copy().start()

    @pl.when(i < n_tiles)
    def _():
        @pl.when(i > 0)
        def _():
            x_copy(i).wait()

        start = pl.multiple_of(i * ts, ts)
        xn = _layernorm_cols(
            x_v[:, pl.ds(start, ts)].astype(jnp.float32)).astype(jnp.bfloat16)
        qkv = jnp.dot(wqkvt_s[...], xn, preferred_element_type=jnp.float32)
        qk = qkv[:2 * d]
        pqk = (jnp.where(qk > 0, qk + 1.0, jnp.exp(qk)) + _PHI_EPS).astype(jnp.bfloat16)
        v = qkv[2 * d:].astype(jnp.bfloat16)
        pk = pqk[d:]
        pq_s[:, pl.ds(start, ts)] = pqk[:d]
        for r0, r1, c0, c1 in blocks:
            kvt_s[r0:r1, c0:c1] += lax.dot_general(
                v[r0:r1], pk[c0:c1], _NT, preferred_element_type=jnp.float32)
        zsum_s[...] += lax.dot_general(
            jnp.ones((zsum_s.shape[0], ts), jnp.bfloat16), pk, _NT,
            preferred_element_type=jnp.float32)

    @pl.when(i == n_tiles - 1)
    def _():
        wo_copy().wait()
        for r0, r1, c0, c1 in blocks:
            kvt = kvt_s[r0:r1, c0:c1]
            row = lax.broadcasted_iota(jnp.int32, kvt.shape, 0) + r0
            col = lax.broadcasted_iota(jnp.int32, kvt.shape, 1) + c0
            r = jnp.where(_head_of(row, dh) == _head_of(col, dh), kvt, 0.0)
            mt_s[:, c0:c1] = lax.dot_general(
                wo_v[r0:r1, :], r.astype(jnp.bfloat16), _TN,
                preferred_element_type=jnp.float32).astype(jnp.bfloat16)
        row = lax.broadcasted_iota(jnp.int32, zt_s.shape, 0)
        col = lax.broadcasted_iota(jnp.int32, zt_s.shape, 1)
        zt_s[...] = jnp.where((row & (heads - 1)) == _head_of(col, dh),
                              zsum_s[0:1, :], 0.0).astype(jnp.bfloat16)

    @pl.when(i >= n_tiles)
    def _():
        @pl.when(i == n_tiles)
        def _():
            w1_copy().wait()
            w2_copy().wait()

        start = pl.multiple_of((i - n_tiles) * ts, ts)
        pq = pq_s[:, pl.ds(start, ts)]
        den = jnp.dot(zt_s[...], pq, preferred_element_type=jnp.float32)
        rec = 1.0 / (den + _DEN_EPS)
        rec_hi = rec.astype(jnp.bfloat16).astype(jnp.float32)
        drow = lax.broadcasted_iota(jnp.int32, den.shape, 0)
        r2 = jnp.where(drow < heads, rec_hi, rec - rec_hi).astype(jnp.bfloat16)
        erow = lax.broadcasted_iota(jnp.int32, (d, pad), 0)
        ecol = lax.broadcasted_iota(jnp.int32, (d, pad), 1)
        expand = jnp.where(_head_of(erow, dh) == (ecol & (heads - 1)),
                           1.0, 0.0).astype(jnp.bfloat16)
        rb = jnp.dot(expand, r2, preferred_element_type=jnp.float32)
        pqs = (pq.astype(jnp.float32) * rb).astype(jnp.bfloat16)
        attn = jnp.dot(mt_s[...], pqs, preferred_element_type=jnp.float32)
        h = x_v[:, pl.ds(start, ts)].astype(jnp.float32) + attn
        prow = lax.broadcasted_iota(jnp.int32, (pad, ts), 0)
        hn_aug = jnp.concatenate(
            [_layernorm_cols(h), jnp.where(prow == 0, 1.0, 0.0)], axis=0)
        hn = hn_aug.T.astype(jnp.bfloat16)
        acc = h + b2_s[:, :1]
        for c in range(f // fc):
            a = jnp.dot(hn, w1_v[:, c * fc:(c + 1) * fc],
                        preferred_element_type=jnp.float32)
            a = jnp.maximum(a, 0.0)
            a = (a * a).astype(jnp.bfloat16)
            acc = acc + lax.dot_general(w2t_v[:, c * fc:(c + 1) * fc], a, _NT,
                                        preferred_element_type=jnp.float32)
        o_ref[...] = acc.astype(o_ref.dtype)


@jax.jit
def pallas_sequential_preLN__linear_attn_block__dense_activation_squared_relu__prompt_kernel(
    A_x: jax.Array,
    A_wqkv: jax.Array,
    A_wo: jax.Array,
    B_x: jax.Array,
    B_w1: jax.Array,
    B_b1: jax.Array,
    B_w2: jax.Array,
    B_b2: jax.Array,
):
    del B_x
    b, s, d = A_x.shape
    assert b == 1
    f = B_w1.shape[1]
    dp = _round_up(d, _LANE)
    assert dp - d == 2 * _NUM_HEADS and d % 16 == 0
    ts = 512
    fc = 512
    assert s % ts == 0 and f % fc == 0
    n_tiles = s // ts
    wqc = 512
    n_wq_chunks = -(-3 * d // wqc)

    xt = A_x.reshape(s, d).T
    w2t = B_w2.T

    kernel = functools.partial(
        _kernel, n_tiles=n_tiles, ts=ts, d=d, dp=dp, f=f, fc=fc, wqc=wqc, heads=_NUM_HEADS)

    hbm = pl.BlockSpec(memory_space=pltpu.HBM)
    out_t = pl.pallas_call(
        kernel,
        grid=(2 * n_tiles,),
        in_specs=[
            pl.BlockSpec((f,), lambda i: (0,)),
            pl.BlockSpec((d,), lambda i: (0,)),
            hbm, hbm, hbm, hbm, hbm,
        ],
        out_specs=pl.BlockSpec((d, ts), lambda i: (0, jnp.maximum(i - n_tiles, 0))),
        out_shape=jax.ShapeDtypeStruct((d, s), A_x.dtype),
        scratch_shapes=[
            pltpu.VMEM((d, s), jnp.bfloat16),
            pltpu.VMEM((d, 3 * d), jnp.bfloat16),
            pltpu.VMEM((d, d), jnp.bfloat16),
            pltpu.VMEM((dp, f), jnp.bfloat16),
            pltpu.VMEM((d, f), jnp.bfloat16),
            pltpu.SemaphoreType.DMA((n_tiles,)),
            pltpu.SemaphoreType.DMA((n_wq_chunks,)),
            pltpu.SemaphoreType.DMA((3,)),
            pltpu.VMEM((3 * d, d), jnp.bfloat16),
            pltpu.VMEM((d, s), jnp.bfloat16),
            pltpu.VMEM((d, d), jnp.float32),
            pltpu.VMEM((16, d), jnp.float32),
            pltpu.VMEM((d, d), jnp.bfloat16),
            pltpu.VMEM((dp - d, d), jnp.bfloat16),
            pltpu.VMEM((d, _LANE), jnp.float32),
        ],
        compiler_params=pltpu.CompilerParams(
            dimension_semantics=("arbitrary",),
            vmem_limit_bytes=100 * 1024 * 1024,
        ),
    )(B_b1, B_b2, xt, A_wqkv, A_wo, B_w1, w2t)
    return out_t.T.reshape(b, s, d)
```

```python
import functools

import jax
import jax.numpy as jnp
from jax import lax
import jax.experimental.pallas as pl
import jax.experimental.pallas.tpu as pltpu

_LN_EPS = 1e-5
_PHI_EPS = 1e-6
_DEN_EPS = 1e-6
_NUM_HEADS = 32
_LANE = 128

_NT = (((1,), (1,)), ((), ()))
_TN = (((0,), (0,)), ((), ()))


def _round_up(a, b):
    return (a + b - 1) // b * b


def _chunks(n, size):
    return [(c, min(c + size, n)) for c in range(0, n, size)]


def _layernorm_cols(x):
    m = jnp.mean(x, axis=0, keepdims=True)
    xc = x - m
    v = jnp.mean(xc * xc, axis=0, keepdims=True)
    return xc * lax.rsqrt(v + _LN_EPS)


def _phi(t):
    return jnp.where(t > 0, t + 1.0, jnp.exp(t)) + _PHI_EPS


def _head_of(idx, dh):
    return jnp.floor((idx.astype(jnp.float32) + 0.5) * (1.0 / dh)).astype(jnp.int32)


def _head_blocks(d, dh):
    blocks = []
    for c0, c1 in _chunks(d, _LANE):
        r0 = (c0 // dh) * dh // 16 * 16
        r1 = min(_round_up(((c1 - 1) // dh + 1) * dh, 16), d)
        blocks.append((r0, r1, c0, c1))
    return blocks


def _kernel(b1_hbm, b2_hbm, x_hbm, wqkv_hbm, wo_hbm, w1_hbm, w2t_hbm, o_hbm,
            b1_v, b2_v, x_v, wqkv_v, wo_v, w1_v, w2t_v, o_v,
            x_sems, wqkv_sems, w_sems, o_sems,
            wqkvt_s, pq_s, kvt_s, zsum_s, mt_s, zt_s, b2_s,
            *, n_tiles, ts, d, dp, f, fc, wq_chunk, out_chunk, heads):
    i = pl.program_id(0)
    dh = d // heads
    pad = dp - d
    blocks = _head_blocks(d, dh)
    wq_chunks = _chunks(3 * d, wq_chunk)
    out_rows = _chunks(d, out_chunk)

    def x_copy(t):
        return pltpu.make_async_copy(
            x_hbm.at[:, pl.ds(t * ts, ts)], x_v.at[:, pl.ds(t * ts, ts)], x_sems.at[t])

    def wqkv_copy(j):
        c0, c1 = wq_chunks[j]
        return pltpu.make_async_copy(
            wqkv_hbm.at[:, pl.ds(c0, c1 - c0)], wqkv_v.at[:, pl.ds(c0, c1 - c0)],
            wqkv_sems.at[j])

    def w1_copy():
        return pltpu.make_async_copy(w1_hbm, w1_v.at[pl.ds(0, d), :], w_sems.at[0])

    def w2_copy():
        return pltpu.make_async_copy(w2t_hbm, w2t_v, w_sems.at[1])

    def wo_copy():
        return pltpu.make_async_copy(wo_hbm, wo_v, w_sems.at[2])

    def b1_copy():
        return pltpu.make_async_copy(b1_hbm, b1_v, w_sems.at[3])

    def b2_copy():
        return pltpu.make_async_copy(b2_hbm, b2_v, w_sems.at[4])

    def out_copy(t, p):
        r0, r1 = out_rows[p]
        rows, cols = pl.ds(r0, r1 - r0), pl.ds(t * ts, ts)
        return pltpu.make_async_copy(
            o_v.at[rows, cols], o_hbm.at[rows, cols], o_sems.at[t, p])

    @pl.when(i == 0)
    def _():
        wqkv_copy(0).start()
        wqkv_copy(1).start()
        b1_copy().start()
        b2_copy().start()
        kvt_s[...] = jnp.zeros(kvt_s.shape, kvt_s.dtype)
        zsum_s[...] = jnp.zeros(zsum_s.shape, zsum_s.dtype)
        for j, (c0, c1) in enumerate(wq_chunks):
            wqkv_copy(j).wait()
            if j + 2 < len(wq_chunks):
                wqkv_copy(j + 2).start()
            if j + 2 == len(wq_chunks):
                x_copy(0).start()
            wqkvt_s[c0:c1, :] = (
                wqkv_v[:, c0:c1].astype(jnp.float32).T.astype(jnp.bfloat16))
        b1_copy().wait()
        b2_copy().wait()
        prow = lax.broadcasted_iota(jnp.int32, (pad, f), 0)
        w1_v[d:, :] = jnp.where(
            prow == 0, b1_v[...].astype(jnp.float32).reshape(1, f), 0.0
        ).astype(jnp.bfloat16)
        b2_s[...] = jnp.broadcast_to(
            b2_v[...].astype(jnp.float32).reshape(1, d), (_LANE, d)).T
        x_copy(0).wait()
        for t in range(1, n_tiles):
            x_copy(t).start()
        wo_copy().start()
        w1_copy().start()
        w2_copy().start()

    @pl.when(i < n_tiles)
    def _():
        @pl.when(i > 0)
        def _():
            x_copy(i).wait()

        start = pl.multiple_of(i * ts, ts)
        xn = _layernorm_cols(
            x_v[:, pl.ds(start, ts)].astype(jnp.float32)).astype(jnp.bfloat16)
        qkv = jnp.dot(wqkvt_s[...], xn, preferred_element_type=jnp.float32)
        pqk = _phi(qkv[:2 * d]).astype(jnp.bfloat16)
        v = qkv[2 * d:].astype(jnp.bfloat16)
        pk = pqk[d:]
        pq_s[:, pl.ds(start, ts)] = pqk[:d]
        for r0, r1, c0, c1 in blocks:
            kvt_s[r0:r1, c0:c1] += lax.dot_general(
                v[r0:r1], pk[c0:c1], _NT, preferred_element_type=jnp.float32)
        zsum_s[...] += lax.dot_general(
            jnp.ones((zsum_s.shape[0], ts), jnp.bfloat16), pk, _NT,
            preferred_element_type=jnp.float32)

    @pl.when(i == n_tiles - 1)
    def _():
        wo_copy().wait()
        for r0, r1, c0, c1 in blocks:
            kvt = kvt_s[r0:r1, c0:c1]
            row = lax.broadcasted_iota(jnp.int32, kvt.shape, 0) + r0
            col = lax.broadcasted_iota(jnp.int32, kvt.shape, 1) + c0
            r = jnp.where(_head_of(row, dh) == _head_of(col, dh), kvt, 0.0)
            mt_s[:, c0:c1] = lax.dot_general(
                wo_v[r0:r1, :], r.astype(jnp.bfloat16), _TN,
                preferred_element_type=jnp.float32).astype(jnp.bfloat16)
        row = lax.broadcasted_iota(jnp.int32, zt_s.shape, 0)
        col = lax.broadcasted_iota(jnp.int32, zt_s.shape, 1)
        zt_s[...] = jnp.where((row & (heads - 1)) == _head_of(col, dh),
                              zsum_s[0:1, :], 0.0).astype(jnp.bfloat16)

    @pl.when(i >= n_tiles)
    def _():
        @pl.when(i == n_tiles)
        def _():
            w1_copy().wait()
            w2_copy().wait()

        t = i - n_tiles
        start = pl.multiple_of(t * ts, ts)
        pq = pq_s[:, pl.ds(start, ts)]
        den = jnp.dot(zt_s[...], pq, preferred_element_type=jnp.float32)
        rec = 1.0 / (den + _DEN_EPS)
        rec_hi = rec.astype(jnp.bfloat16).astype(jnp.float32)
        drow = lax.broadcasted_iota(jnp.int32, den.shape, 0)
        r2 = jnp.where(drow < heads, rec_hi, rec - rec_hi).astype(jnp.bfloat16)
        erow = lax.broadcasted_iota(jnp.int32, (d, pad), 0)
        ecol = lax.broadcasted_iota(jnp.int32, (d, pad), 1)
        expand = jnp.where(_head_of(erow, dh) == (ecol & (heads - 1)),
                           1.0, 0.0).astype(jnp.bfloat16)
        rb = jnp.dot(expand, r2, preferred_element_type=jnp.float32)
        pqs = (pq.astype(jnp.float32) * rb).astype(jnp.bfloat16)
        attn = jnp.dot(mt_s[...], pqs, preferred_element_type=jnp.float32)
        h = x_v[:, pl.ds(start, ts)].astype(jnp.float32) + attn
        prow = lax.broadcasted_iota(jnp.int32, (pad, ts), 0)
        hn_aug = jnp.concatenate(
            [_layernorm_cols(h), jnp.where(prow == 0, 1.0, 0.0)], axis=0)
        hn = hn_aug.T.astype(jnp.bfloat16)

        def act(c):
            a = jnp.dot(hn, w1_v[:, c * fc:(c + 1) * fc],
                        preferred_element_type=jnp.float32)
            a = jnp.maximum(a, 0.0)
            return (a * a).astype(jnp.bfloat16)

        acc = h + b2_s[:, :1]
        last = f // fc - 1
        for c in range(last):
            acc = acc + lax.dot_general(w2t_v[:, c * fc:(c + 1) * fc], act(c), _NT,
                                        preferred_element_type=jnp.float32)
        a = act(last)
        for p, (r0, r1) in enumerate(out_rows):
            res = acc[r0:r1] + lax.dot_general(
                w2t_v[r0:r1, last * fc:(last + 1) * fc], a, _NT,
                preferred_element_type=jnp.float32)
            o_v[r0:r1, pl.ds(start, ts)] = res.astype(o_v.dtype)
            out_copy(t, p).start()

        @pl.when(t == n_tiles - 1)
        def _():
            for tt in range(n_tiles):
                for p in range(len(out_rows)):
                    out_copy(tt, p).wait()


@jax.jit
def pallas_sequential_preLN__linear_attn_block__dense_activation_squared_relu__prompt_kernel(
    A_x: jax.Array,
    A_wqkv: jax.Array,
    A_wo: jax.Array,
    B_x: jax.Array,
    B_w1: jax.Array,
    B_b1: jax.Array,
    B_w2: jax.Array,
    B_b2: jax.Array,
):
    del B_x
    b, s, d = A_x.shape
    f = B_w1.shape[1]
    dp = _round_up(d, _LANE)
    ts = 512
    fc = 512
    wq_chunk = 512
    out_chunk = 192
    assert b == 1 and dp - d == 2 * _NUM_HEADS and d % 16 == 0
    assert s % ts == 0 and f % fc == 0 and out_chunk % 16 == 0
    n_tiles = s // ts
    n_wq = len(_chunks(3 * d, wq_chunk))
    n_out = len(_chunks(d, out_chunk))
    assert n_wq >= 2

    xt = A_x.reshape(s, d).T
    w2t = B_w2.T

    kernel = functools.partial(
        _kernel, n_tiles=n_tiles, ts=ts, d=d, dp=dp, f=f, fc=fc,
        wq_chunk=wq_chunk, out_chunk=out_chunk, heads=_NUM_HEADS)

    hbm = pl.BlockSpec(memory_space=pltpu.HBM)
    bf16 = jnp.bfloat16
    out_t = pl.pallas_call(
        kernel,
        grid=(2 * n_tiles,),
        in_specs=[hbm] * 7,
        out_specs=hbm,
        out_shape=jax.ShapeDtypeStruct((d, s), A_x.dtype),
        scratch_shapes=[
            pltpu.VMEM((f,), bf16),
            pltpu.VMEM((d,), bf16),
            pltpu.VMEM((d, s), bf16),
            pltpu.VMEM((d, 3 * d), bf16),
            pltpu.VMEM((d, d), bf16),
            pltpu.VMEM((dp, f), bf16),
            pltpu.VMEM((d, f), bf16),
            pltpu.VMEM((d, s), A_x.dtype),
            pltpu.SemaphoreType.DMA((n_tiles,)),
            pltpu.SemaphoreType.DMA((n_wq,)),
            pltpu.SemaphoreType.DMA((5,)),
            pltpu.SemaphoreType.DMA((n_tiles, n_out)),
            pltpu.VMEM((3 * d, d), bf16),
            pltpu.VMEM((d, s), bf16),
            pltpu.VMEM((d, d), jnp.float32),
            pltpu.VMEM((16, d), jnp.float32),
            pltpu.VMEM((d, d), bf16),
            pltpu.VMEM((dp - d, d), bf16),
            pltpu.VMEM((d, _LANE), jnp.float32),
        ],
        compiler_params=pltpu.CompilerParams(
            dimension_semantics=("arbitrary",),
            vmem_limit_bytes=100 * 1024 * 1024,
        ),
    )(B_b1, B_b2, xt, A_wqkv, A_wo, B_w1, w2t)
    return out_t.T.reshape(b, s, d)
```
